```python
import jax
import jax.numpy as jnp

def _softmax(x, axis=-1):
    return jax.nn.softmax(x, axis=axis)
def _gelu(x):
    return jax.nn.gelu(x, approximate=True)
def _silu(x):
    return jax.nn.silu(x)
def _sigmoid(x):
    return jax.nn.sigmoid(x)
def _layernorm(x, axis=-1, eps=1e-5):
    m = jnp.mean(x, axis=axis, keepdims=True)
    v = jnp.var(x, axis=axis, keepdims=True)
    return (x - m) / jnp.sqrt(v + eps)
def _scatter_add(tgt, idx, src, axis=0):
    return tgt.at[idx].add(src)
def _segment_sum(src, seg, n):
    return jax.ops.segment_sum(src, seg, n)
class _Rng:
    def __init__(self, key):
        self._k = key
    def _next(self):
        self._k, sub = jax.random.split(self._k)
        return sub
    def normal(self, shape):
        return jax.random.normal(self._next(), shape, dtype=jnp.bfloat16)
    def randint(self, lo, hi, shape):
        return jax.random.randint(self._next(), shape, lo, hi, dtype=jnp.int32)
    def uniform(self, shape, lo=0.0, hi=1.0):
        return jax.random.uniform(self._next(), shape, jnp.bfloat16, lo, hi)
    def permutation(self, n):
        return jax.random.permutation(self._next(), n)


kernel_name = 'gated_mix__compressed_kv_cla__ssm_conv_h3__prompt'

def setup_inputs():
    _rng = _Rng(jax.random.key(int.from_bytes(__import__("os").urandom(4), "little")))
    _w = (lambda a: (lambda t: t.astype(jnp.bfloat16) if jnp.issubdtype(t.dtype, jnp.floating) else t)(jnp.asarray(a)))
    def _A_setup():
        B, H, Sq, Sk, D, M = 1, 32, 2048, 2048, 128, 1024
        Dc = 4 * D
        return {
            "x": _w((lambda *s: _rng.normal(s) * 0.05)(B, Sq, M)),
            "c_kv": _w((lambda *s: _rng.normal(s) * 0.05)(B, Sk, Dc)),
            "w_q": _w((lambda *s: _rng.normal(s) * 0.05)(M, H, D) * (M ** -0.5)),
            "w_uk": _w((lambda *s: _rng.normal(s) * 0.05)(Dc, H, D) * (Dc ** -0.5)),
            "w_uv": _w((lambda *s: _rng.normal(s) * 0.05)(Dc, H, D) * (Dc ** -0.5)),
            "w_o": _w((lambda *s: _rng.normal(s) * 0.05)(H, D, M) * ((H * D) ** -0.5)),
        }
    _A_in = _A_setup()

    def _B_setup():
        B, S, D = 1, 2048, 1024
        ks = 4
        return {
            "q": _w((lambda *s: _rng.normal(s) * 0.05)(B, S, D)),
            "k": _w((lambda *s: _rng.normal(s) * 0.05)(B, S, D)),
            "v": _w((lambda *s: _rng.normal(s) * 0.05)(B, S, D)),
            "shift_k": _w((lambda *s: _rng.normal(s) * 0.05)(D, ks) * 0.5),
            "ssm_k": _w((lambda *s: _rng.normal(s) * 0.05)(D, S) * (1.0 / S ** 0.5)),
            "ssm_D": _w((lambda *s: _rng.normal(s) * 0.05)(D)),
        }
    _B_in = _B_setup()

    return {
        "A_x": _A_in["x"],
        "A_c_kv": _A_in["c_kv"],
        "A_w_q": _A_in["w_q"],
        "A_w_uk": _A_in["w_uk"],
        "A_w_uv": _A_in["w_uv"],
        "A_w_o": _A_in["w_o"],
        "B_q": _B_in["q"],
        "B_k": _B_in["k"],
        "B_v": _B_in["v"],
        "B_shift_k": _B_in["shift_k"],
        "B_ssm_k": _B_in["ssm_k"],
        "B_ssm_D": _B_in["ssm_D"],
        "gate_w": _w((lambda *s: _rng.normal(s) * 0.05)(1024)),
    }

def reference(A_x, A_c_kv, A_w_q, A_w_uk, A_w_uv, A_w_o, B_q, B_k, B_v, B_shift_k, B_ssm_k, B_ssm_D, gate_w):
    def _A_ref(x, c_kv, w_q, w_uk, w_uv, w_o):
        B, Sq, M = x.shape[0], x.shape[1], x.shape[2]
        Sk = c_kv.shape[1]
        H, D = w_q.shape[1], w_q.shape[2]
        q = jnp.einsum("bqm,mhd->bhqd", x, w_q)
        k = jnp.einsum("bkc,chd->bhkd", c_kv, w_uk)
        v = jnp.einsum("bkc,chd->bhkd", c_kv, w_uv)
        scores = jnp.einsum("bhqd,bhkd->bhqk", q, k) * (D ** -0.5)
        off = Sk - Sq
        qi = jnp.arange(Sq)[:, None]
        kj = jnp.arange(Sk)[None, :]
        cmask = kj <= (qi + off)
        scores = jnp.where(cmask[None, None], scores, -1e9)
        p = _softmax(scores, axis=-1)
        ctx = jnp.einsum("bhqk,bhkd->bhqd", p, v)
        return jnp.einsum("bhqd,hdm->bqm", ctx, w_o)

    def _B_ref(q, k, v, shift_k, ssm_k, ssm_D):
        B, S, D = q.shape
        ks = shift_k.shape[-1]
        k_pad = jnp.pad(k, ((0, 0), (ks - 1, 0), (0, 0)))
        k_shift = jnp.zeros_like(k)
        for t in range(ks):
            k_shift = k_shift + k_pad[:, t:t + S, :] * shift_k[:, ks - 1 - t][None, None, :]
        kv = k_shift * v
        L = 2 * S
        kv_pad = jnp.pad(kv, ((0, 0), (0, S), (0, 0)))
        kf_pad = jnp.pad(ssm_k, ((0, 0), (0, S)))
        kv_f = (lambda x, axes=(-2,-1): jnp.fft.rfft2(x.astype(jnp.float32), axes=axes))(kv_pad[:, None, :, :], axes=(1, 2))
        kf_f = (lambda x, axes=(-2,-1): jnp.fft.rfft2(x.astype(jnp.float32), axes=axes))(kf_pad[:, None, :], axes=(1, 2))
        kf_f = (lambda x, *d: x.transpose(*d))(kf_f, 1, 2, 0)
        y_f = kv_f * kf_f[None, :, :, :]
        y = (lambda x, s, axes=(-2,-1): jnp.fft.irfft2(x, s=s, axes=axes).astype(jnp.bfloat16))(y_f, (1, L), axes=(1, 2))[:, 0, :S, :]
        y = y + kv * ssm_D[None, None, :]
        return q * y

    x = A_x
    g = _sigmoid((x * gate_w).sum(-1, keepdims=True))
    a = _A_ref(x, A_c_kv, A_w_q, A_w_uk, A_w_uv, A_w_o)
    b = _B_ref(x, B_k, B_v, B_shift_k, B_ssm_k, B_ssm_D)
    return g * a + (1 - g) * b
```

```python
import math

import jax
import jax.numpy as jnp
import numpy as np
import jax.experimental.pallas as pl
import jax.experimental.pallas.tpu as pltpu
from jax import lax

S, M, H, D, DC = 2048, 1024, 32, 128, 512
C = 128
NC = S // C
BQ = 128
F32, BF16 = jnp.float32, jnp.bfloat16


def _dft_mats():
    n = np.arange(C)[None, :]
    f = np.arange(C)[:, None]
    th = np.pi * (2 * f + 1) * n / (2 * C)
    fwd = np.concatenate([np.cos(th), -np.sin(th)], 0)
    inv = np.concatenate([np.cos(th).T, -np.sin(th).T], 1) / C
    return fwd.astype(np.float32), inv.astype(np.float32)


_FWD, _INV = _dft_mats()
_NT = (((1,), (1,)), ((), ()))


def _dot(a, b):
    return jnp.dot(a, b, preferred_element_type=F32)


def _kernel(x_h, c_h, wq_h, wk_h, wv_h, wo_h, k_h, v_h, sh_ref, sk_h, sd_ref, gw_ref,
            f_ref, g_ref, o_h,
            x_v, c_v, wq_v, wk_v, wv_v, wo_v, ctx_v, u_v, U_v, H_v,
            kb, vb, sb, kp, q_s, k_s, v_s, ob, sems, bsem, osem):
    def bcopies(i, slot):
        r = pl.ds(pl.multiple_of(i * C, C), C)
        return (pltpu.make_async_copy(k_h.at[r], kb.at[slot], bsem.at[0, slot]),
                pltpu.make_async_copy(v_h.at[r], vb.at[slot], bsem.at[1, slot]),
                pltpu.make_async_copy(sk_h.at[:, r], sb.at[slot], bsem.at[2, slot]))

    for cp in bcopies(0, 0):
        cp.start()
    big = [pltpu.make_async_copy(s, d, sems.at[n]) for n, (s, d) in enumerate(
        [(c_h, c_v), (wk_h, wk_v.bitcast(BF16)), (wv_h, wv_v.bitcast(BF16)), (x_h, x_v), (wq_h, wq_v.bitcast(BF16)), (wo_h, wo_v)])]
    for cp in big:
        cp.start()

    lane = lax.broadcasted_iota(jnp.int32, (M, 128), 1)
    sh = jnp.where(lane < 4, sh_ref[...], 0.0).T[:8]
    kp[0:8, :] = jnp.zeros((8, M), F32)
    U_v[NC] = jnp.zeros((2 * C, M), F32)
    sign = (1 - 2 * (lax.broadcasted_iota(jnp.int32, (C, M), 0) & 1)).astype(F32)

    def b1(i, _):
        slot = i % 2

        @pl.when(i + 1 < NC)
        def _():
            for cp in bcopies(i + 1, 1 - slot):
                cp.start()
        for cp in bcopies(i, slot):
            cp.wait()
        kp[8:8 + C, :] = kb[slot].astype(F32)
        ks = kp[8:8 + C, :] * sh[0:1]
        for t in range(1, 4):
            ks = ks + kp[8 - t:8 - t + C, :] * sh[t:t + 1]
        kp[0:8, :] = kp[C:C + 8, :]
        u = (ks * vb[slot].astype(F32)).astype(BF16)
        u_v[pl.ds(pl.multiple_of(i * C, C), C), :] = u
        U_v[i] = _dot(f_ref[...], u)
        H_v[i] = lax.dot_general(f_ref[...], sb[slot], _NT, preferred_element_type=F32)
        return 0
    lax.fori_loop(0, NC, b1, 0)

    def hfix(t, _):
        j = NC - 1 - t
        p = H_v[j - 1]
        H_v[j, :C] = H_v[j, :C] - sign * p[C:]
        H_v[j, C:] = H_v[j, C:] + sign * p[:C]
        return 0
    lax.fori_loop(0, NC - 1, hfix, 0)

    for cp in big[:5]:
        cp.wait()

    qscale = D ** -0.5 * math.log2(math.e)
    ri = lax.broadcasted_iota(jnp.int32, (BQ, BQ), 0)
    ci = lax.broadcasted_iota(jnp.int32, (BQ, BQ), 1)
    tri = ci <= ri

    def getw(ref, n, j):
        w = ref[pl.ds(j, n, stride=H // 2), :]
        lo = lax.bitcast_convert_type(w << 16, F32).astype(BF16)
        hi = lax.bitcast_convert_type(w & jnp.int32(-65536), F32).astype(BF16)
        return lo, hi

    def pair(j, _):
        wq, wk, wv = getw(wq_v, M, j), getw(wk_v, DC, j), getw(wv_v, DC, j)
        for e in range(2):
            q_s[e] = (_dot(x_v[...], wq[e]) * qscale).astype(BF16)
            k_s[e] = _dot(c_v[...], wk[e]).astype(BF16)
            v_s[e] = _dot(c_v[...], wv[e]).astype(BF16)
        for e in range(2):
            col = pl.ds(pl.multiple_of((2 * j + e) * D, D), D)
            for i in range(S // BQ):
                L = (i + 1) * BQ
                q = q_s[e, i * BQ:L, :]
                sd = lax.dot_general(q, k_s[e, L - BQ:L, :], _NT, preferred_element_type=F32)
                s = jnp.where(tri, sd, -1e30)
                if i:
                    so = lax.dot_general(q, k_s[e, :L - BQ, :], _NT, preferred_element_type=F32)
                    s = jnp.concatenate([so, s], 1)
                m = jnp.max(s, axis=1, keepdims=True)
                p = jnp.exp2(s - m)
                l = jnp.sum(p, axis=1, keepdims=True)
                o = _dot(p.astype(BF16), v_s[e, :L, :])
                ctx_v[i * BQ:L, col] = (o * (1.0 / l)).astype(BF16)
        return 0
    lax.fori_loop(0, H // 2, pair, 0)

    big[5].wait()

    def ocopy(i, slot):
        return pltpu.make_async_copy(
            ob.at[slot], o_h.at[pl.ds(pl.multiple_of(i * C, C), C)], osem.at[slot])

    def fin(i, _):
        slot = i % 2
        r = pl.ds(pl.multiple_of(i * C, C), C)
        a = _dot(ctx_v[r, :], wo_v[...])
        yr = jnp.zeros((C, M), F32)
        yi = jnp.zeros((C, M), F32)
        for j in range(NC):
            n = jnp.where(i >= j, i - j, NC)
            ur, ui = U_v[n, :C], U_v[n, C:]
            hr, hi = H_v[j, :C], H_v[j, C:]
            yr = yr + (hr * ur - hi * ui)
            yi = yi + (hr * ui + hi * ur)
        y = _dot(g_ref[...], jnp.concatenate([yr, yi], 0).astype(BF16))
        y = y + u_v[r, :].astype(F32) * sd_ref[...].astype(F32)
        xx = x_v[r, :].astype(F32)
        g = jax.nn.sigmoid(jnp.sum(xx * gw_ref[...].astype(F32), axis=1, keepdims=True))
        res = g * a + (1.0 - g) * (xx * y)

        @pl.when(i >= 2)
        def _():
            ocopy(i - 2, slot).wait()
        ob[slot] = res.astype(BF16)
        ocopy(i, slot).start()
        return 0
    lax.fori_loop(0, NC, fin, 0)
    ocopy(NC - 2, 0).wait()
    ocopy(NC - 1, 1).wait()


@jax.jit
def pallas_gated_mix__compressed_kv_cla__ssm_conv_h3__prompt_kernel(
    A_x, A_c_kv, A_w_q, A_w_uk, A_w_uv, A_w_o, B_q, B_k, B_v, B_shift_k, B_ssm_k, B_ssm_D, gate_w,
):
    del B_q
    any_ = pl.BlockSpec(memory_space=pl.ANY)
    vm = pl.BlockSpec(memory_space=pltpu.VMEM)
    V = pltpu.VMEM
    out = pl.pallas_call(
        _kernel,
        out_shape=jax.ShapeDtypeStruct((S, M), BF16),
        in_specs=[any_] * 8 + [vm, any_, vm, vm, vm, vm],
        out_specs=any_,
        scratch_shapes=[
            V((S, M), BF16), V((S, DC), BF16), V((M * H // 2, D), jnp.int32), V((DC * H // 2, D), jnp.int32),
            V((DC * H // 2, D), jnp.int32), V((H * D, M), BF16), V((S, H * D), BF16), V((S, M), BF16),
            V((NC + 1, 2 * C, M), F32), V((NC, 2 * C, M), F32),
            V((2, C, M), BF16), V((2, C, M), BF16), V((2, M, C), BF16), V((8 + C, M), F32),
            V((2, S, D), BF16), V((2, S, D), BF16), V((2, S, D), BF16), V((2, C, M), BF16),
            pltpu.SemaphoreType.DMA((6,)), pltpu.SemaphoreType.DMA((3, 2)),
            pltpu.SemaphoreType.DMA((2,)),
        ],
        compiler_params=pltpu.CompilerParams(vmem_limit_bytes=120 * 1024 * 1024),
    )(
        A_x.reshape(S, M), A_c_kv.reshape(S, DC), A_w_q.reshape(M * H, D),
        A_w_uk.reshape(DC * H, D), A_w_uv.reshape(DC * H, D), A_w_o.reshape(H * D, M),
        B_k.reshape(S, M), B_v.reshape(S, M), jnp.pad(B_shift_k.astype(F32), ((0, 0), (0, 124))), B_ssm_k,
        B_ssm_D.reshape(1, M), gate_w.reshape(1, M),
        jnp.asarray(_FWD, BF16), jnp.asarray(_INV, BF16),
    )
    return out.reshape(1, S, M)
```

```python
import math

import jax
import jax.numpy as jnp
import numpy as np
import jax.experimental.pallas as pl
import jax.experimental.pallas.tpu as pltpu
from jax import lax

S, M, H, D, DC = 2048, 1024, 32, 128, 512
C = 128
NC = S // C
BQ = 128
PR = 2048
F32, BF16 = jnp.float32, jnp.bfloat16


def _dft_mats():
    n = np.arange(C)[None, :]
    f = np.arange(C)[:, None]
    th = np.pi * (2 * f + 1) * n / (2 * C)
    fwd = np.concatenate([np.cos(th), -np.sin(th)], 0)
    inv = np.concatenate([np.cos(th).T, -np.sin(th).T], 1) / C
    return fwd.astype(np.float32), inv.astype(np.float32)


_FWD, _INV = _dft_mats()
_NT = (((1,), (1,)), ((), ()))


def _dot(a, b):
    return jnp.dot(a, b, preferred_element_type=F32)


def _kernel(x_h, c_h, wq_h, wk_h, wv_h, wo_h, k_h, v_h, sh_ref, sk_h, sd_ref, gw_ref,
            f_ref, g_ref, o_h,
            x_v, c_v, wq_v, wk_v, wv_v, wo_v, ctx_v, u_v, U_v, H_v,
            kb, vb, sb, kp, q_s, k_s, v_s, ob, s_s, y_s, a_s, w_s, sems, bsem, osem):
    def bcopies(i, slot):
        r = pl.ds(pl.multiple_of(i * C, C), C)
        return (pltpu.make_async_copy(k_h.at[r], kb.at[slot], bsem.at[0, slot]),
                pltpu.make_async_copy(v_h.at[r], vb.at[slot], bsem.at[1, slot]),
                pltpu.make_async_copy(sk_h.at[:, r], sb.at[slot], bsem.at[2, slot]))

    for cp in bcopies(0, 0):
        cp.start()
    big = [pltpu.make_async_copy(s, d, sems.at[n]) for n, (s, d) in enumerate(
        [(c_h, c_v), (wk_h, wk_v.bitcast(BF16)), (wv_h, wv_v.bitcast(BF16)), (x_h, x_v), (wq_h, wq_v.bitcast(BF16))] + [(wo_h.at[:, t * 128:(t + 1) * 128], wo_v.at[t]) for t in range(8)])]
    for cp in big[:5]:
        cp.start()

    lane = lax.broadcasted_iota(jnp.int32, (M, 128), 1)
    sh = jnp.where(lane < 4, sh_ref[...], 0.0).T[:8]
    kp[0:8, :] = jnp.zeros((8, M), F32)
    U_v[NC] = jnp.zeros((2 * C, M), F32)
    sign = (1 - 2 * (lax.broadcasted_iota(jnp.int32, (C, M), 0) & 1)).astype(F32)

    def b1(i, _):
        slot = i % 2

        @pl.when(i + 1 < NC)
        def _():
            for cp in bcopies(i + 1, 1 - slot):
                cp.start()
        for cp in bcopies(i, slot):
            cp.wait()
        kp[8:8 + C, :] = kb[slot].astype(F32)
        ks = kp[8:8 + C, :] * sh[0:1]
        for t in range(1, 4):
            ks = ks + kp[8 - t:8 - t + C, :] * sh[t:t + 1]
        kp[0:8, :] = kp[C:C + 8, :]
        u = (ks * vb[slot].astype(F32)).astype(BF16)
        u_v[pl.ds(pl.multiple_of(i * C, C), C), :] = u
        U_v[i] = _dot(f_ref[...], u)
        H_v[i] = lax.dot_general(f_ref[...], sb[slot], _NT, preferred_element_type=F32)
        return 0
    with jax.named_scope("pB1"):
        lax.fori_loop(0, NC, b1, 0)

    def hfix(t, _):
        j = NC - 1 - t
        p = H_v[j - 1]
        H_v[j, :C] = H_v[j, :C] - sign * p[C:]
        H_v[j, C:] = H_v[j, C:] + sign * p[:C]
        return 0
    with jax.named_scope("pHfix"):
        lax.fori_loop(0, NC - 1, hfix, 0)

    with jax.named_scope("pWait"):
        for cp in big[:5]:
            cp.wait()

    for cp in big[5:]:
        cp.start()

    qscale = D ** -0.5 * math.log2(math.e)
    ri = lax.broadcasted_iota(jnp.int32, (BQ, BQ), 0)
    ci = lax.broadcasted_iota(jnp.int32, (BQ, BQ), 1)
    tri = ci <= ri

    def getw(ref, n, j):
        w = ref[pl.ds(j, n, stride=H // 2), :]
        lo = lax.bitcast_convert_type(w << 16, F32).astype(BF16)
        hi = lax.bitcast_convert_type(w & jnp.int32(-65536), F32).astype(BF16)
        return lo, hi

    def proj(j):
        o = 2 * (j % 2)
        w_s[:M] = jnp.concatenate(getw(wq_v, M, j), 1)
        w_s[M:M + DC] = jnp.concatenate(getw(wk_v, DC, j), 1)
        w_s[M + DC:] = jnp.concatenate(getw(wv_v, DC, j), 1)
        for r in range(S // PR):
            r = slice(r * PR, (r + 1) * PR)
            for dst, val in ((q_s, _dot(x_v[r, :], w_s[:M]) * qscale),
                             (k_s, _dot(c_v[r, :], w_s[M:M + DC])),
                             (v_s, _dot(c_v[r, :], w_s[M + DC:]))):
                dst[o, r, :] = val[:, :D].astype(BF16)
                dst[o + 1, r, :] = val[:, D:].astype(BF16)
            yield

    def pair(j, last):
        gen = iter(()) if last else proj(j + 1)
        o_ = 2 * (j % 2)
        blocks = [(e, i) for e in range(2) for i in (range(NC) if e == 0 else reversed(range(NC)))]

        def qk(n, t, mx):
            e, i = blocks[n]
            s = lax.dot_general(q_s[o_ + e, i * BQ:(i + 1) * BQ, :], k_s[o_ + e, t * BQ:(t + 1) * BQ, :],
                                _NT, preferred_element_type=F32)
            if t == i:
                s = jnp.where(tri, s, -1e30)
            s_s[n % 2, t] = s
            return s if mx is None else jnp.maximum(mx, s)

        mx = None
        for t in range(blocks[0][1] + 1):
            mx = qk(0, t, mx)
        for n, (e, i) in enumerate(blocks):
            m = jnp.max(mx, axis=1, keepdims=True)
            mx = o = l = None
            nxt = blocks[n + 1][1] + 1 if n + 1 < len(blocks) else 0
            for t in range(max(i + 1, nxt)):
                if t < nxt:
                    mx = qk(n + 1, t, mx)
                if t <= i:
                    p = jnp.exp2(s_s[n % 2, t] - m)
                    l = p if l is None else l + p
                    pv = _dot(p.astype(BF16), v_s[o_ + e, t * BQ:(t + 1) * BQ, :])
                    o = pv if o is None else o + pv
            col = pl.ds(pl.multiple_of((2 * j + e) * D, D), D)
            ctx_v[i * BQ:(i + 1) * BQ, col] = (
                o * (1.0 / jnp.sum(l, axis=1, keepdims=True))).astype(BF16)
            if n % (PR // 64) == PR // 64 - 1:
                next(gen, None)
        return 0
    with jax.named_scope("pA"):
        list(proj(0))
        lax.fori_loop(0, H // 2 - 1, lambda j, _: pair(j, False), 0)
        pair(H // 2 - 1, True)

    for cp in big[5:]:
        cp.wait()

    def ocopy(i, slot):
        return pltpu.make_async_copy(
            ob.at[slot], o_h.at[pl.ds(pl.multiple_of(i * 2 * C, 2 * C), 2 * C)], osem.at[slot])

    def fin(i, _):
        slot = i % 2
        r = pl.ds(pl.multiple_of(i * 2 * C, 2 * C), 2 * C)
        ns = [jnp.where(2 * i + 1 >= j, 2 * i + 1 - j, NC) for j in range(NC + 1)]
        def step(t, _):
            a_s[t] = _dot(ctx_v[r, :], wo_v[t])
            r0 = pl.ds(pl.multiple_of(t * 16, 16), 16)
            r1 = pl.ds(pl.multiple_of(C + t * 16, 16), 16)
            for nt in range(8):
                ln = slice(nt * 128, (nt + 1) * 128)
                acc, hs = [None] * 4, {}
                for j in range(NC + 1):
                    ur, ui = U_v[ns[j], r0, ln], U_v[ns[j], r1, ln]
                    if j < NC:
                        hs[j] = H_v[j, r0, ln], H_v[j, r1, ln]
                    for w, jj in ((0, j - 1), (2, j)):
                        if 0 <= jj < NC:
                            hr, hi = hs[jj]
                            pr, pi = hr * ur - hi * ui, hr * ui + hi * ur
                            acc[w] = pr if acc[w] is None else acc[w] + pr
                            acc[w + 1] = pi if acc[w + 1] is None else acc[w + 1] + pi
                for w in range(2):
                    y_s[w, r0, ln] = acc[2 * w].astype(BF16)
                    y_s[w, r1, ln] = acc[2 * w + 1].astype(BF16)
            return 0
        lax.fori_loop(0, 8, step, 0)
        a = jnp.concatenate([a_s[t] for t in range(8)], 1)
        y = jnp.concatenate([_dot(g_ref[...], y_s[w]) for w in range(2)], 0)
        y = y + u_v[r, :].astype(F32) * sd_ref[...].astype(F32)
        xx = x_v[r, :].astype(F32)
        g = jax.nn.sigmoid(jnp.sum(xx * gw_ref[...].astype(F32), axis=1, keepdims=True))
        res = g * a + (1.0 - g) * (xx * y)

        @pl.when(i >= 2)
        def _():
            ocopy(i - 2, slot).wait()
        ob[slot] = res.astype(BF16)
        ocopy(i, slot).start()
        return 0
    with jax.named_scope("pC"):
        lax.fori_loop(0, NC // 2, fin, 0)
    ocopy(NC // 2 - 2, 0).wait()
    ocopy(NC // 2 - 1, 1).wait()


@jax.jit
def pallas_gated_mix__compressed_kv_cla__ssm_conv_h3__prompt_kernel(
    A_x, A_c_kv, A_w_q, A_w_uk, A_w_uv, A_w_o, B_q, B_k, B_v, B_shift_k, B_ssm_k, B_ssm_D, gate_w,
):
    del B_q
    any_ = pl.BlockSpec(memory_space=pl.ANY)
    vm = pl.BlockSpec(memory_space=pltpu.VMEM)
    V = pltpu.VMEM
    out = pl.pallas_call(
        _kernel,
        out_shape=jax.ShapeDtypeStruct((S, M), BF16),
        in_specs=[any_] * 8 + [vm, any_, vm, vm, vm, vm],
        out_specs=any_,
        scratch_shapes=[
            V((S, M), BF16), V((S, DC), BF16), V((M * H // 2, D), jnp.int32), V((DC * H // 2, D), jnp.int32),
            V((DC * H // 2, D), jnp.int32), V((8, H * D, 128), BF16), V((S, H * D), BF16), V((S, M), BF16),
            V((NC + 1, 2 * C, M), F32), V((NC, 2 * C, M), F32),
            V((2, C, M), BF16), V((2, C, M), BF16), V((2, M, C), BF16), V((8 + C, M), F32),
            V((4, S, D), BF16), V((4, S, D), BF16), V((4, S, D), BF16), V((2, 2 * C, M), BF16),
            V((2, NC, BQ, BQ), F32), V((2, 2 * C, M), BF16), V((8, 2 * C, 128), F32), V((2 * M, 2 * D), BF16),
            pltpu.SemaphoreType.DMA((13,)), pltpu.SemaphoreType.DMA((3, 2)),
            pltpu.SemaphoreType.DMA((2,)),
        ],
        compiler_params=pltpu.CompilerParams(vmem_limit_bytes=127 * 1024 * 1024),
    )(
        A_x.reshape(S, M), A_c_kv.reshape(S, DC), A_w_q.reshape(M * H, D),
        A_w_uk.reshape(DC * H, D), A_w_uv.reshape(DC * H, D), A_w_o.reshape(H * D, M),
        B_k.reshape(S, M), B_v.reshape(S, M), jnp.pad(B_shift_k.astype(F32), ((0, 0), (0, 124))), B_ssm_k,
        B_ssm_D.reshape(1, M), gate_w.reshape(1, M),
        jnp.asarray(_FWD, BF16), jnp.asarray(_INV, BF16),
    )
    return out.reshape(1, S, M)
```

```python
import math

import jax
import jax.numpy as jnp
import numpy as np
import jax.experimental.pallas as pl
import jax.experimental.pallas.tpu as pltpu
from jax import lax

S, M, H, D, DC = 2048, 1024, 32, 128, 512
C = 128
NC = S // C
BQ = 128
F32, BF16 = jnp.float32, jnp.bfloat16


def _dft_mats():
    n = np.arange(C)[None, :]
    f = np.arange(C)[:, None]
    th = np.pi * (2 * f + 1) * n / (2 * C)
    fwd = np.concatenate([np.cos(th), -np.sin(th)], 0)
    inv = np.concatenate([np.cos(th).T, -np.sin(th).T], 1) / C
    return fwd.astype(np.float32), inv.astype(np.float32)


_FWD, _INV = _dft_mats()
_NT = (((1,), (1,)), ((), ()))


def _dot(a, b):
    return jnp.dot(a, b, preferred_element_type=F32)


def _kernel(x_h, c_h, wq_h, wk_h, wv_h, wo_h, k_h, v_h, sh_ref, sk_h, sd_ref, gw_ref,
            f_ref, g_ref, o_h,
            x_v, c_v, wq_v, wk_v, wv_v, wo_v, ctx_v, u_v, U_v, H_v,
            kb, vb, sb, kp, q_s, k_s, v_s, ob, s_s, y_s, a_s, sems, bsem, osem):
    def bcopies(i, slot):
        r = pl.ds(pl.multiple_of(i * C, C), C)
        return (pltpu.make_async_copy(k_h.at[r], kb.at[slot], bsem.at[0, slot]),
                pltpu.make_async_copy(v_h.at[r], vb.at[slot], bsem.at[1, slot]),
                pltpu.make_async_copy(sk_h.at[:, r], sb.at[slot], bsem.at[2, slot]))

    for cp in bcopies(0, 0):
        cp.start()
    big = [pltpu.make_async_copy(s, d, sems.at[n]) for n, (s, d) in enumerate(
        [(c_h, c_v), (wk_h, wk_v.bitcast(BF16)), (wv_h, wv_v.bitcast(BF16)), (x_h, x_v), (wq_h, wq_v.bitcast(BF16))] + [(wo_h.at[:, t * 128:(t + 1) * 128], wo_v.at[t]) for t in range(8)])]
    big[0].start()

    lane = lax.broadcasted_iota(jnp.int32, (M, 128), 1)
    sh = jnp.where(lane < 4, sh_ref[...], 0.0).T[:8]
    kp[0:8, :] = jnp.zeros((8, M), F32)
    U_v[NC] = jnp.zeros((2 * C, M), F32)
    sign = (1 - 2 * (lax.broadcasted_iota(jnp.int32, (C, M), 0) & 1)).astype(F32)

    def b1(i, _):
        slot = i % 2

        @pl.when(i + 1 < NC)
        def _():
            for cp in bcopies(i + 1, 1 - slot):
                cp.start()
        for n in range(1, 5):
            pl.when(i == 2 * n - 1)(big[n].start)
        for cp in bcopies(i, slot):
            cp.wait()
        kp[8:8 + C, :] = kb[slot].astype(F32)
        ks = kp[8:8 + C, :] * sh[0:1]
        for t in range(1, 4):
            ks = ks + kp[8 - t:8 - t + C, :] * sh[t:t + 1]
        kp[0:8, :] = kp[C:C + 8, :]
        u = (ks * vb[slot].astype(F32)).astype(BF16)
        u_v[pl.ds(pl.multiple_of(i * C, C), C), :] = u
        U_v[i] = _dot(f_ref[...], u)
        H_v[i] = lax.dot_general(f_ref[...], sb[slot], _NT, preferred_element_type=F32)
        return 0
    with jax.named_scope("pB1"):
        lax.fori_loop(0, NC, b1, 0)

    def hfix(t, _):
        j = NC - 1 - t
        p = H_v[j - 1]
        H_v[j, :C] = H_v[j, :C] - sign * p[C:]
        H_v[j, C:] = H_v[j, C:] + sign * p[:C]
        return 0
    with jax.named_scope("pHfix"):
        lax.fori_loop(0, NC - 1, hfix, 0)

    with jax.named_scope("pWait"):
        for cp in big[:5]:
            cp.wait()

    for cp in big[5:]:
        cp.start()

    qscale = D ** -0.5 * math.log2(math.e)
    ri = lax.broadcasted_iota(jnp.int32, (BQ, BQ), 0)
    ci = lax.broadcasted_iota(jnp.int32, (BQ, BQ), 1)
    tri = ci <= ri

    def getw(ref, n, j):
        w = ref[pl.ds(j, n, stride=H // 2), :]
        lo = lax.bitcast_convert_type(w << 16, F32).astype(BF16)
        hi = lax.bitcast_convert_type(w & jnp.int32(-65536), F32).astype(BF16)
        return lo, hi

    def pair(j, _):
        wq, wk, wv = getw(wq_v, M, j), getw(wk_v, DC, j), getw(wv_v, DC, j)
        for e in range(2):
            q_s[e] = (_dot(x_v[...], wq[e]) * qscale).astype(BF16)
            k_s[e] = _dot(c_v[...], wk[e]).astype(BF16)
            v_s[e] = _dot(c_v[...], wv[e]).astype(BF16)
        blocks = [(e, i) for e in range(2) for i in (range(NC) if e == 0 else reversed(range(NC)))]

        def qk(n, t, mx):
            e, i = blocks[n]
            s = lax.dot_general(q_s[e, i * BQ:(i + 1) * BQ, :], k_s[e, t * BQ:(t + 1) * BQ, :],
                                _NT, preferred_element_type=F32)
            if t == i:
                s = jnp.where(tri, s, -1e30)
            s_s[n % 2, t] = s
            return s if mx is None else jnp.maximum(mx, s)

        mx = None
        for t in range(blocks[0][1] + 1):
            mx = qk(0, t, mx)
        for n, (e, i) in enumerate(blocks):
            m = jnp.max(mx, axis=1, keepdims=True)
            mx = o = l = None
            nxt = blocks[n + 1][1] + 1 if n + 1 < len(blocks) else 0
            for t in range(max(i + 1, nxt)):
                if t < nxt:
                    mx = qk(n + 1, t, mx)
                if t <= i:
                    p = jnp.exp2(s_s[n % 2, t] - m)
                    pb = p.astype(BF16)
                    l = p if l is None else l + p
                    if t == i:
                        pb = jnp.where(l >= 0, p, 0.).astype(BF16)
                    pv = _dot(pb, v_s[e, t * BQ:(t + 1) * BQ, :])
                    o = pv if o is None else o + pv
            col = pl.ds(pl.multiple_of((2 * j + e) * D, D), D)
            ctx_v[i * BQ:(i + 1) * BQ, col] = (
                o * (1.0 / jnp.sum(l, axis=1, keepdims=True))).astype(BF16)
        return 0
    with jax.named_scope("pA"):
        lax.fori_loop(0, H // 2, pair, 0)

    for cp in big[5:]:
        cp.wait()

    def ocopy(i, slot):
        return pltpu.make_async_copy(
            ob.at[slot], o_h.at[pl.ds(pl.multiple_of(i * 2 * C, 2 * C), 2 * C)], osem.at[slot])

    def fin(i, nj):
        slot = i % 2
        r = pl.ds(pl.multiple_of(i * 2 * C, 2 * C), 2 * C)
        ns = [jnp.where(2 * i + 1 >= j, 2 * i + 1 - j, NC) for j in range(NC + 1)]
        def step(t, _):
            a_s[t] = _dot(ctx_v[r, :], wo_v[t])
            r0 = pl.ds(pl.multiple_of(t * 16, 16), 16)
            r1 = pl.ds(pl.multiple_of(C + t * 16, 16), 16)
            for nt in range(8):
                ln = slice(nt * 128, (nt + 1) * 128)
                acc, hs = [None] * 4, {}
                for j in range(nj):
                    ur, ui = U_v[ns[j], r0, ln], U_v[ns[j], r1, ln]
                    if j < nj:
                        hs[j] = H_v[j, r0, ln], H_v[j, r1, ln]
                    for w, jj in ((0, j - 1), (2, j)):
                        if 0 <= jj < nj:
                            hr, hi = hs[jj]
                            pr, pi = hr * ur - hi * ui, hr * ui + hi * ur
                            acc[w] = pr if acc[w] is None else acc[w] + pr
                            acc[w + 1] = pi if acc[w + 1] is None else acc[w + 1] + pi
                for w in range(2):
                    y_s[w, r0, ln] = acc[2 * w].astype(BF16)
                    y_s[w, r1, ln] = acc[2 * w + 1].astype(BF16)
            return 0
        lax.fori_loop(0, 8, step, 0)
        a = jnp.concatenate([a_s[t] for t in range(8)], 1)
        y = jnp.concatenate([_dot(g_ref[...], y_s[w]) for w in range(2)], 0)
        y = y + u_v[r, :].astype(F32) * sd_ref[...].astype(F32)
        xx = x_v[r, :].astype(F32)
        g = jax.nn.sigmoid(jnp.sum(xx * gw_ref[...].astype(F32), axis=1, keepdims=True))
        res = g * a + (1.0 - g) * (xx * y)

        @pl.when(i >= 2)
        def _():
            ocopy(i - 2, slot).wait()
        ob[slot] = res.astype(BF16)
        ocopy(i, slot).start()
        return 0
    with jax.named_scope("pC"):
        for z in range(4):
            lax.fori_loop(2 * z, 2 * z + 2, lambda i, _, z=z: fin(i, 4 * z + 4), 0)
    ocopy(NC // 2 - 2, 0).wait()
    ocopy(NC // 2 - 1, 1).wait()


@jax.jit
def pallas_gated_mix__compressed_kv_cla__ssm_conv_h3__prompt_kernel(
    A_x, A_c_kv, A_w_q, A_w_uk, A_w_uv, A_w_o, B_q, B_k, B_v, B_shift_k, B_ssm_k, B_ssm_D, gate_w,
):
    del B_q
    any_ = pl.BlockSpec(memory_space=pl.ANY)
    vm = pl.BlockSpec(memory_space=pltpu.VMEM)
    V = pltpu.VMEM
    out = pl.pallas_call(
        _kernel,
        out_shape=jax.ShapeDtypeStruct((S, M), BF16),
        in_specs=[any_] * 8 + [vm, any_, vm, vm, vm, vm],
        out_specs=any_,
        scratch_shapes=[
            V((S, M), BF16), V((S, DC), BF16), V((M * H // 2, D), jnp.int32), V((DC * H // 2, D), jnp.int32),
            V((DC * H // 2, D), jnp.int32), V((8, H * D, 128), BF16), V((S, H * D), BF16), V((S, M), BF16),
            V((NC + 1, 2 * C, M), F32), V((NC, 2 * C, M), F32),
            V((2, C, M), BF16), V((2, C, M), BF16), V((2, M, C), BF16), V((8 + C, M), F32),
            V((2, S, D), BF16), V((2, S, D), BF16), V((2, S, D), BF16), V((2, 2 * C, M), BF16),
            V((2, NC, BQ, BQ), F32), V((2, 2 * C, M), BF16), V((8, 2 * C, 128), F32),
            pltpu.SemaphoreType.DMA((13,)), pltpu.SemaphoreType.DMA((3, 2)),
            pltpu.SemaphoreType.DMA((2,)),
        ],
        compiler_params=pltpu.CompilerParams(vmem_limit_bytes=127 * 1024 * 1024),
    )(
        A_x.reshape(S, M), A_c_kv.reshape(S, DC), A_w_q.reshape(M * H, D),
        A_w_uk.reshape(DC * H, D), A_w_uv.reshape(DC * H, D), A_w_o.reshape(H * D, M),
        B_k.reshape(S, M), B_v.reshape(S, M), jnp.pad(B_shift_k.astype(F32), ((0, 0), (0, 124))), B_ssm_k,
        B_ssm_D.reshape(1, M), gate_w.reshape(1, M),
        jnp.asarray(_FWD, BF16), jnp.asarray(_INV, BF16),
    )
    return out.reshape(1, S, M)
```
